```python
import os as _os
_os.environ.setdefault("JAX_PLATFORMS", "cpu")
import jax
import jax.numpy as jnp

def _softmax(x, axis=-1):
    return jax.nn.softmax(x, axis=axis)
def _gelu(x):
    return jax.nn.gelu(x, approximate=True)
def _silu(x):
    return jax.nn.silu(x)
def _sigmoid(x):
    return jax.nn.sigmoid(x)
def _layernorm(x, axis=-1, eps=1e-5):
    m = jnp.mean(x, axis=axis, keepdims=True)
    v = jnp.var(x, axis=axis, keepdims=True)
    return (x - m) / jnp.sqrt(v + eps)
def _scatter_add(tgt, idx, src, axis=0):
    return tgt.at[idx].add(src)
def _segment_sum(src, seg, n):
    return jax.ops.segment_sum(src, seg, n)
class _Rng:
    def __init__(self, key):
        self._k = key
    def _next(self):
        self._k, sub = jax.random.split(self._k)
        return sub
    def normal(self, shape):
        return jax.random.normal(self._next(), shape, dtype=jnp.bfloat16)
    def randint(self, lo, hi, shape):
        return jax.random.randint(self._next(), shape, lo, hi, dtype=jnp.int32)
    def uniform(self, shape, lo=0.0, hi=1.0):
        return jax.random.uniform(self._next(), shape, jnp.bfloat16, lo, hi)
    def permutation(self, n):
        return jax.random.permutation(self._next(), n)


kernel_name = 'concat_heads__sliding_block_cached__sliding_block_cached__decode'

def setup_inputs():
    _rng = _Rng(jax.random.key(int.from_bytes(__import__("os").urandom(4), "little")))
    _w = (lambda a: (lambda t: t.astype(jnp.bfloat16) if jnp.issubdtype(t.dtype, jnp.floating) else t)(jnp.asarray(a)))
    def _A_setup():
        B, Sq, D = 1, 1, 640
        Hq, Hkv, Sk, Dh = 32, 32, 4096, 192
        assert Hq % Hkv == 0, (Hq, Hkv)
        return {
            "x": _w((lambda *s: _rng.normal(s) * 0.8)(B, Sq, D)),
            "k_cache": _w((lambda *s: _rng.normal(s) * 0.8)(B, Hkv, Sk, Dh)),
            "v_cache": _w((lambda *s: _rng.normal(s) * 0.05)(B, Hkv, Sk, Dh)),
            "wq": _w((lambda *s: _rng.normal(s) * 0.8)(D, Hq * Dh) * (D ** -0.5)),
            "wo": _w((lambda *s: _rng.normal(s) * 0.05)(Hq * Dh, D) * ((Hq * Dh) ** -0.5)),
        }
    _A_in = _A_setup()

    def _B_setup():
        B, Sq, D = 1, 1, 640
        Hq, Hkv, Sk, Dh = 32, 32, 4096, 192
        assert Hq % Hkv == 0, (Hq, Hkv)
        return {
            "x": _w((lambda *s: _rng.normal(s) * 0.8)(B, Sq, D)),
            "k_cache": _w((lambda *s: _rng.normal(s) * 0.8)(B, Hkv, Sk, Dh)),
            "v_cache": _w((lambda *s: _rng.normal(s) * 0.05)(B, Hkv, Sk, Dh)),
            "wq": _w((lambda *s: _rng.normal(s) * 0.8)(D, Hq * Dh) * (D ** -0.5)),
            "wo": _w((lambda *s: _rng.normal(s) * 0.05)(Hq * Dh, D) * ((Hq * Dh) ** -0.5)),
        }
    _B_in = _B_setup()

    return {
        "A_x": _A_in["x"],
        "A_k_cache": _A_in["k_cache"],
        "A_v_cache": _A_in["v_cache"],
        "A_wq": _A_in["wq"],
        "A_wo": _A_in["wo"],
        "B_x": _B_in["x"],
        "B_k_cache": _B_in["k_cache"],
        "B_v_cache": _B_in["v_cache"],
        "B_wq": _B_in["wq"],
        "B_wo": _B_in["wo"],
    }

def reference(A_x, A_k_cache, A_v_cache, A_wq, A_wo, B_x, B_k_cache, B_v_cache, B_wq, B_wo):
    def _A_ref(x, k_cache, v_cache, wq, wo):
        B, Sq, D = x.shape
        Hq, Dh = 32, 192
        Hkv, Sk = k_cache.shape[1], k_cache.shape[2]
        W = min(4096, max(256, Sk // 4))
        rep = Hq // Hkv
        q = (lambda x, *d: x.transpose(*d))((x @ wq).reshape(B, Sq, Hq, Dh), 0, 2, 1, 3)
        k = jnp.repeat(k_cache[:, :, Sk - W:, :], rep, axis=1)
        v = jnp.repeat(v_cache[:, :, Sk - W:, :], rep, axis=1)
        scores = jnp.einsum("bhqd,bhkd->bhqk", q, k) * (Dh ** -0.5)
        p = _softmax(scores, axis=-1)
        o = jnp.einsum("bhqk,bhkd->bhqd", p, v)
        return (lambda x, *d: x.transpose(*d))(o, 0, 2, 1, 3).reshape(B, Sq, Hq * Dh) @ wo

    def _B_ref(x, k_cache, v_cache, wq, wo):
        B, Sq, D = x.shape
        Hq, Dh = 32, 192
        Hkv, Sk = k_cache.shape[1], k_cache.shape[2]
        W = min(4096, max(256, Sk // 4))
        rep = Hq // Hkv
        q = (lambda x, *d: x.transpose(*d))((x @ wq).reshape(B, Sq, Hq, Dh), 0, 2, 1, 3)
        k = jnp.repeat(k_cache[:, :, Sk - W:, :], rep, axis=1)
        v = jnp.repeat(v_cache[:, :, Sk - W:, :], rep, axis=1)
        scores = jnp.einsum("bhqd,bhkd->bhqk", q, k) * (Dh ** -0.5)
        p = _softmax(scores, axis=-1)
        o = jnp.einsum("bhqk,bhkd->bhqd", p, v)
        return (lambda x, *d: x.transpose(*d))(o, 0, 2, 1, 3).reshape(B, Sq, Hq * Dh) @ wo

    a = _A_ref(A_x, A_k_cache, A_v_cache, A_wq, A_wo)
    b = _B_ref(B_x, B_k_cache, B_v_cache, B_wq, B_wo)
    return jnp.concatenate([a, b], axis=-1)
```

```python
import jax
import jax.numpy as jnp
import jax.experimental.pallas as pl
import jax.experimental.pallas.tpu as pltpu

_HQ, _DH = 32, 192
_G = 8


@jax.jit
def pallas_concat_heads__sliding_block_cached__sliding_block_cached__decode_kernel(
    A_x: jax.Array,
    A_k_cache: jax.Array,
    A_v_cache: jax.Array,
    A_wq: jax.Array,
    A_wo: jax.Array,
    B_x: jax.Array,
    B_k_cache: jax.Array,
    B_v_cache: jax.Array,
    B_wq: jax.Array,
    B_wo: jax.Array,
):
    _, _, d_model = A_x.shape
    sk = A_k_cache.shape[2]
    w = min(4096, max(256, sk // 4))
    n_groups = _HQ // _G
    gd = _G * _DH
    scale = _DH**-0.5
    dtype = A_x.dtype

    def kernel(
        ax, ak, av, awq, awo, bx, bk, bv, bwq, bwo, out_ref,
        x_buf, k_buf, v_buf, wq_buf, wo_buf, sems,
    ):
        x_hbm, k_hbm, v_hbm = (ax, bx), (ak, bk), (av, bv)
        wq_hbm, wo_hbm = (awq, bwq), (awo, bwo)

        copies = {}

        def plan(key, src, dst):
            copies[key] = pltpu.make_async_copy(src, dst, sems.at[len(copies)])

        for b in range(2):
            for g in range(n_groups):
                rows = pl.ds(g * gd, gd)
                win = pl.ds(sk - w, w)
                plan(("wq", b, g), wq_hbm[b].at[:, rows], wq_buf.at[b, g])
                if g == 0:
                    plan(("x", b), x_hbm[b], x_buf.at[b])
                plan(("k", b, g), k_hbm[b].at[rows, win], k_buf.at[b, g])
                plan(("v", b, g), v_hbm[b].at[rows, win], v_buf.at[b, g])
                plan(("wo", b, g), wo_hbm[b].at[rows, :], wo_buf.at[b, g])
        for c in copies.values():
            c.start()

        head = jax.lax.broadcasted_iota(jnp.int32, (_G, gd), 0)
        col = jax.lax.broadcasted_iota(jnp.int32, (_G, gd), 1)
        own = jnp.logical_and(col >= head * _DH, col < (head + 1) * _DH)

        for b in range(2):
            acc = jnp.zeros((_G, d_model), jnp.float32)
            for g in range(n_groups):
                copies["wq", b, g].wait()
                if g == 0:
                    copies["x", b].wait()
                x = jnp.broadcast_to(x_buf[b], (_G, d_model))
                q = jnp.dot(x, wq_buf[b, g], preferred_element_type=jnp.float32)
                q = jnp.where(own, q, 0.0).astype(dtype)

                copies["k", b, g].wait()
                s = jnp.dot(q, k_buf[b, g], preferred_element_type=jnp.float32)
                s = s * scale
                e = jnp.exp(s - jnp.max(s, axis=-1, keepdims=True))
                inv = 1.0 / jnp.sum(e, axis=-1, keepdims=True)

                copies["v", b, g].wait()
                o = jax.lax.dot_general(
                    e.astype(dtype), v_buf[b, g], (((1,), (1,)), ((), ())),
                    preferred_element_type=jnp.float32,
                )
                o = jnp.where(own, o * inv, 0.0).astype(dtype)

                copies["wo", b, g].wait()
                acc += jnp.dot(o, wo_buf[b, g], preferred_element_type=jnp.float32)
            out_ref[:, b * d_model:(b + 1) * d_model] = jnp.sum(
                acc, axis=0, keepdims=True
            ).astype(out_ref.dtype)

    def seq_minor(cache):
        return jnp.swapaxes(cache, 2, 3).reshape(_HQ * _DH, sk)

    out = pl.pallas_call(
        kernel,
        out_shape=jax.ShapeDtypeStruct((1, 2 * d_model), dtype),
        in_specs=[pl.BlockSpec(memory_space=pltpu.HBM)] * 10,
        out_specs=pl.BlockSpec(memory_space=pltpu.VMEM),
        scratch_shapes=[
            pltpu.VMEM((2, 1, d_model), dtype),
            pltpu.VMEM((2, n_groups, gd, w), dtype),
            pltpu.VMEM((2, n_groups, gd, w), dtype),
            pltpu.VMEM((2, n_groups, d_model, gd), dtype),
            pltpu.VMEM((2, n_groups, gd, d_model), dtype),
            pltpu.SemaphoreType.DMA((2 * (4 * n_groups + 1),)),
        ],
        compiler_params=pltpu.CompilerParams(vmem_limit_bytes=110 * 1024 * 1024),
    )(
        A_x.reshape(1, d_model), seq_minor(A_k_cache), seq_minor(A_v_cache), A_wq, A_wo,
        B_x.reshape(1, d_model), seq_minor(B_k_cache), seq_minor(B_v_cache), B_wq, B_wo,
    )
    return out.reshape(1, 1, 2 * d_model)
```

```python
import jax
import jax.numpy as jnp
from jax import lax
import jax.experimental.pallas as pl
import jax.experimental.pallas.tpu as pltpu

_HQ, _DH = 32, 192
_F32 = jnp.float32


def make(name="k2", pad=128, compute="qsoyt", bounds=False, flags=None, pace=20):
    lead = 24

    def fn(A_x, A_k_cache, A_v_cache, A_wq, A_wo, B_x, B_k_cache, B_v_cache, B_wq, B_wo):
        d_model = A_x.shape[-1]
        sk = A_k_cache.shape[2]
        w = min(4096, max(256, sk // 4))
        scale = _DH**-0.5
        dtype = A_x.dtype

        def kernel(
            ax, ak, av, awq, awo, bx, bk, bv, bwq, bwo, out_ref,
            x_buf, wq_buf, kv_buf, woa_buf, wob_buf, q_buf, e_buf, r_buf, o_buf, sems,
        ):
            X, WQ, KV, WOA, WOB = 0, 1, 3, 7, 8

            def start(src, dst, sem, q):
                pltpu.make_async_copy(src, dst, sems.at[sem]).start(priority=q)

            def split(n1, n0, g, q):
                return pl.ds((n1 + n0) * g, n1) if q else pl.ds((n1 + n0) * g + n1, n0)

            def wq_stream(b, src):
                def copy(c, g, q):
                    idx = (split(4, 1, g, q), c >> 1, pl.ds(8 * (c & 1), 8))
                    start(src.at[idx], wq_buf.at[(b, *idx)], WQ + b, q)
                return copy, 3, 32

            def kv_stream(j, src):
                def copy(c, g, q):
                    r, rows = split(3, 1, g, q), pl.ds(pl.multiple_of(8 * c, 8), 8)
                    start(src.at[r, rows, pl.ds(sk - w, w)],
                          kv_buf.at[j, r, rows, pl.ds(0, w)], KV + j, q)
                return copy, 24, 8

            def woa_copy(c, g, q):
                idx = (split(4, 1, g, q), pl.ds(8 * c, 8))
                start(awo.at[idx], woa_buf.at[idx], WOA, q)

            def wob_piece(r, t, sem, q):
                start(bwo.at[r, t], wob_buf.at[r, t], sem, q)

            def wob_stage(j):
                def copy(c, g, q):
                    wob_piece(split(3, 1, g, q), pl.ds(80 * j + 8 * c, 8), WOB + j, q)
                return copy, 3, 10

            def wob_tail1(g):
                def copy(c, _, q):
                    wob_piece(split(3, 1, g, q), pl.ds(240 + 8 * c, 8), WOB + 3 + g, q)
                return copy, 1, 10

            def wob_tail2(c, _, q):
                wob_piece(pl.ds(8, 2) if q else pl.ds(10, 1), pl.ds(240 + 8 * c, 8), WOB + 5, q)

            def wob_tail3(c, _, q):
                wob_piece(pl.ds(11, 1), pl.ds(240 + 2 * c, 2), WOB + 6, q)

            streams = [
                wq_stream(0, awq), wq_stream(1, bwq),
                kv_stream(0, ak), kv_stream(1, bk), kv_stream(2, av), kv_stream(3, bv),
                (woa_copy, 3, 32), wob_stage(0), wob_stage(1), wob_stage(2),
                wob_tail1(0), wob_tail1(1), (wob_tail2, 1, 10), (wob_tail3, 1, lead),
            ]

            def locate(pos, n):
                for copy, per_col, cols in streams:
                    if pos < per_col * cols:
                        assert pos + n <= per_col * cols, (pos, n, per_col * cols)
                        return copy, per_col, pos
                    pos -= per_col * cols
                raise AssertionError

            cursor = [0]

            def position(per_col, p0, per, i, u):
                if isinstance(i, int):
                    return divmod(p0 + i * per + u, per_col)
                if per % per_col == 0:
                    return (p0 + u) // per_col + i * (per // per_col), (p0 + u) % per_col
                assert per_col % per == 0 and p0 % per == 0, (per_col, per, p0)
                m = per_col // per
                j = p0 // per + i
                assert m & (m - 1) == 0
                return j >> (m.bit_length() - 1), (j & (m - 1)) * per + u

            def run(trips, per, work=None, carry=None, tag=""):
                short = locate(cursor[0], trips * per)
                long_ = locate(cursor[0] + lead, trips * per)
                cursor[0] += trips * per

                def body(i, carry):
                    count = [0]

                    def issue():
                        for q, (copy, per_col, p0) in ((1, long_), (0, short)):
                            copy(*position(per_col, p0, per, i, count[0]), q)
                        count[0] += 1

                    if work is not None and tag in compute:
                        carry = work(i, carry, issue)
                    while count[0] < per:
                        issue()
                    return carry

                if trips == 1:
                    return body(0, carry)
                return lax.fori_loop(0, trips, body, carry)

            def wait(view, sem):
                pltpu.make_async_copy(view, view, sems.at[sem]).wait()

            row = lax.broadcasted_iota(jnp.int32, (8, 128), 0)
            lane = lax.broadcasted_iota(jnp.int32, (8, 128), 1)

            def own(t):
                d = lane + 128 * t - _DH * row
                return jnp.logical_and(d >= 0, d < _DH)

            def mod12(t):
                return t - 12 * ((t * 43) >> 9)

            def q_work(b):
                def work(i, carry, issue):
                    x = jnp.broadcast_to(x_buf[b], (8, d_model))
                    wt = wq_buf[b, :, :, i].reshape(80, 3, 8, 128)
                    for u in range(3):
                        issue()
                        q = jnp.dot(x, wt[:, u].reshape(d_model, 128),
                                    preferred_element_type=_F32)
                        t = 16 * u + i
                        q_buf[b, t] = jnp.where(own(mod12(t)), q, 0.0)
                    return carry
                return work

            def s_work(b, g):
                def work(i, s, issue):
                    t = 12 * g + i
                    q = q_buf[b, t].astype(dtype)
                    parts = []
                    for h in range(2):
                        issue()
                        kt = kv_buf[b, pl.ds(2 * t, 2), :, 512 * h:512 * (h + 1)]
                        parts.append(jnp.dot(
                            q, kt.reshape(128, 512), preferred_element_type=_F32))
                    return s + jnp.concatenate(parts, axis=1)
                return work

            def softmax(b, g, s):
                s = s * scale
                e = jnp.exp(s - jnp.max(s, axis=-1, keepdims=True))
                e_buf[b, g] = e
                r_buf[b, g] = jnp.broadcast_to(
                    1.0 / jnp.sum(e, axis=-1, keepdims=True), (8, 128))

            def o_work(b, n, base=0):
                def work(i, carry, issue):
                    t0 = base + n * i
                    g = (t0 * 43) >> 9
                    e = e_buf[b, g].astype(dtype)
                    for u in range(n):
                        t = t0 + u
                        o = 0.0
                        for h in range(2 // n):
                            issue()
                            cols = slice(512 * h, 512 * (h + n))
                            vt = kv_buf[2 + b, pl.ds(2 * t, 2), :, cols].reshape(128, 512 * n)
                            o = o + lax.dot_general(
                                e[:, cols], vt, (((1,), (1,)), ((), ())),
                                preferred_element_type=_F32)
                        o = jnp.where(own(t - 12 * g), o * r_buf[b, g], 0.0)
                        o_buf[b, t] = jnp.broadcast_to(
                            jnp.sum(o, axis=0, keepdims=True), (8, 128))
                    return carry
                return work

            def project(o, wt, acc):
                wt = wt.reshape(16, 5, 8, 128)
                wt = jnp.concatenate(
                    [wt[:, n].reshape(128, 128) for n in range(5)], axis=1)
                return acc + jnp.dot(o.astype(dtype), wt, preferred_element_type=_F32)

            def project_a(big, j, acc):
                r, t = divmod(80 * j, 256)
                n = min(80, 256 - t)
                wt = woa_buf[5 * big + r, t:t + n]
                if n < 80:
                    wt = jnp.concatenate([wt, woa_buf[5 * big + r + 1, 0:80 - n]], axis=0)
                return project(o_buf[0, 16 * big + j], wt, acc)

            def project_b(r, j, acc):
                return project(o_buf[1, 4 * r + j], wob_buf[r, pl.ds(80 * j, 80)], acc)

            def ya_work(j0, n, per):
                def work(i, acc, issue):
                    for u in range(n):
                        if u * per // n != (u - 1) * per // n:
                            issue()
                        acc = project_a(i, j0 + u, acc)
                    return acc
                return work

            def yb_work(j, r0, n):
                def work(i, acc, issue):
                    for u in range(n):
                        if u < 2:
                            issue()
                        acc = project_b(r0 + n * i + u, j, acc)
                    return acc
                return work

            first = streams[0][0]
            for p in range(lead):
                first(p // 3, p % 3, 1)
                if p == 0:
                    start(ax, x_buf.at[0], X, 0)
                    start(bx, x_buf.at[1], X, 0)

            def kv_wait(j):
                wait(kv_buf.at[j, :, :, pl.ds(0, w)], KV + j)

            run(24, 3)
            run(8, 3)
            run(8, 3)
            wait(x_buf, X)
            wait(wq_buf.at[0], WQ)
            run(16, 3, q_work(0), tag="q")
            run(8, 3)
            run(8, 3)
            wait(wq_buf.at[1], WQ + 1)
            run(16, 3, q_work(1), tag="q")
            run(32, 3)
            run(8, 3)
            for b in range(2):
                run(8, 3)
                kv_wait(b)
                for g in range(4):
                    s = run(12, 3, s_work(b, g), jnp.zeros((8, w), _F32), tag="s")
                    if "s" in compute:
                        softmax(b, g, s)
                run(8, 3)
            run(8, 3)
            kv_wait(2)
            run(48, 3, o_work(0, 1), tag="o")
            run(8, 3)
            run(5, 3)
            kv_wait(3)
            run(19, 3, o_work(1, 2), tag="o")
            run(5, 3, o_work(1, 2, 38), tag="o")
            run(3, 3)
            zero = jnp.zeros((8, d_model), _F32)
            run(2, 3)
            run(2, 3)
            wait(woa_buf, WOA)
            acc = run(3, 6, ya_work(0, 8, 6), zero, tag="y")
            run(2, 3)
            acc = run(3, 6, ya_work(8, 8, 6), acc, tag="y")
            out_ref[:, 0:d_model] = acc[0:1].astype(dtype)
            wait(wob_buf.at[:, pl.ds(0, 80)], WOB)
            acc = run(2, 3, yb_work(0, 0, 3), zero, tag="y")
            acc = run(2, 3, yb_work(0, 6, 3), acc, tag="y")
            run(3, 3)
            run(1, 1)
            wait(wob_buf.at[:, pl.ds(80, 80)], WOB + 1)
            acc = run(3, 3, yb_work(1, 0, 3), acc, tag="y")
            run(1, 1)
            acc = run(1, 3, yb_work(1, 9, 3), acc, tag="y")
            run(1, 1)
            run(6, 1)
            run(4, 1)
            wait(wob_buf.at[:, pl.ds(160, 80)], WOB + 2)
            acc = run(5, 2, yb_work(2, 0, 2), acc, tag="y")
            acc = run(1, 2, yb_work(2, 10, 2), acc, tag="y")
            wait(wob_buf.at[pl.ds(0, 4), pl.ds(240, 80)], WOB + 3)
            acc = run(2, 2, yb_work(3, 0, 2), acc, tag="y")
            run(4, 1)
            wob_piece(pl.ds(11, 1), pl.ds(240 + 2 * lead, 80 - 2 * lead), WOB + 6, 1)
            wait(wob_buf.at[pl.ds(4, 4), pl.ds(240, 80)], WOB + 4)
            if "t" in compute:
                for r in range(4, 8):
                    acc = project_b(r, 3, acc)
            wait(wob_buf.at[pl.ds(8, 3), pl.ds(240, 80)], WOB + 5)
            if "t" in compute:
                for r in range(8, 11):
                    acc = project_b(r, 3, acc)
            wait(wob_buf.at[pl.ds(11, 1), pl.ds(240, 80)], WOB + 6)
            if "t" in compute:
                acc = project_b(11, 3, acc)
            out_ref[:, d_model:] = acc[0:1].astype(dtype)

        def cache_view(cache):
            return jnp.swapaxes(cache, 2, 3).reshape(96, 64, sk)

        def tiles(a, *shape):
            r, c = a.shape
            return a.reshape(r // 8, 8, c // 128, 128).transpose(0, 2, 1, 3).reshape(
                *shape, 8, 128)

        out = pl.pallas_call(
            kernel,
            out_shape=jax.ShapeDtypeStruct((1, 2 * d_model), dtype),
            in_specs=[pl.BlockSpec(memory_space=pltpu.HBM)] * 10,
            out_specs=pl.BlockSpec(memory_space=pltpu.VMEM),
            scratch_shapes=[
                pltpu.VMEM((2, 1, d_model), dtype),
                pltpu.VMEM((2, 15, 16, 16, 8, 128), dtype),
                pltpu.VMEM((4, 96, 64, w + pad), dtype),
                pltpu.VMEM((15, 256, 8, 128), dtype),
                pltpu.VMEM((12, 320, 8, 128), dtype),
                pltpu.VMEM((2, 48, 8, 128), _F32),
                pltpu.VMEM((2, 4, 8, w), _F32),
                pltpu.VMEM((2, 4, 8, 128), _F32),
                pltpu.VMEM((2, 48, 8, 128), _F32),
                pltpu.SemaphoreType.DMA((15,)),
            ],
            compiler_params=pltpu.CompilerParams(
                vmem_limit_bytes=110 * 1024 * 1024, disable_bounds_checks=not bounds,
                flags=flags),
            name=name,
        )(
            A_x.reshape(1, d_model), cache_view(A_k_cache), cache_view(A_v_cache),
            tiles(A_wq, 15, 16, 16), tiles(A_wo, 15, 256),
            B_x.reshape(1, d_model), cache_view(B_k_cache), cache_view(B_v_cache),
            tiles(B_wq, 15, 16, 16), tiles(B_wo, 12, 320),
        )
        return out.reshape(1, 1, 2 * d_model)

    return fn


pallas_concat_heads__sliding_block_cached__sliding_block_cached__decode_kernel = jax.jit(make())
```

```python
import functools

import jax
import jax.numpy as jnp
from jax import lax
import jax.experimental.pallas as pl
import jax.experimental.pallas.tpu as pltpu

_HEADS, _HEAD_DIM = 32, 192
_F32 = jnp.float32

_LEAD = 8

_ROWS = ((0, 2, 4, 6), (8, 10, 12, 14), (1, 3, 5, 7), (9, 11, 13))
_LATE_ROWS = ((0, 2, 6, 8), (10, 12, 1, 3), (5, 7, 11, 13))


def _div6(i):
    return (i * 43) >> 8


def _on_queue(queue, pieces):
    return pieces[1:] if queue else pieces[:1]


def _wait(view, sem):
    pltpu.make_async_copy(view, view, sem).wait()


def _side_by_side(tiles, n):
    tiles = tiles.reshape(16, n, 8, 128)
    return jnp.concatenate([tiles[:, j].reshape(128, 128) for j in range(n)], axis=1)


class _Feed:
    def __init__(self, streams):
        self.streams = streams
        self.pos = 0

    def _locate(self, pos):
        for copy, beats, sweeps in self.streams:
            if pos < beats * sweeps:
                return copy, beats, pos, beats * sweeps - pos
            pos -= beats * sweeps
        return None

    def _issue(self, pos, queue):
        place = self._locate(pos)
        if place is not None:
            copy, beats, p, _ = place
            copy(p // beats, p % beats, queue)

    def prime(self):
        for pos in range(_LEAD):
            self._issue(pos, 1)

    def step(self, n=1):
        for _ in range(n):
            self._issue(self.pos + _LEAD, 1)
            self._issue(self.pos, 0)
            self.pos += 1

    def trip(self, trips, per_trip, work=None):
        places = ((1, self._locate(self.pos + _LEAD)), (0, self._locate(self.pos)))
        for _, (_, beats, _, left) in places:
            assert per_trip % beats == 0 and left >= trips * per_trip
        self.pos += trips * per_trip

        def body(i, carry):
            issued = 0

            def step():
                nonlocal issued
                for queue, (copy, beats, p, _) in places:
                    p += issued
                    copy(p // beats + i * (per_trip // beats), p % beats, queue)
                issued += 1

            if work is not None:
                carry = work(i, carry, step)
            assert issued <= per_trip
            while issued < per_trip:
                step()
            return carry

        return body

    def loop(self, trips, per_trip, work=None, carry=None):
        return lax.fori_loop(0, trips, self.trip(trips, per_trip, work), carry)

    def done(self):
        return self._locate(self.pos) is None


def _attend(
    ax, ak, av, awq, awo, bx, bk, bv, bwq, bwo, out_ref,
    x_buf, wq_buf, kv_buf, wo_buf, q_buf, e_buf, inv_buf, o_buf,
    x_sem, wq_sem, kv_sem, wo_sem, end_sem,
):
    dtype = x_buf.dtype
    d_model = x_buf.shape[-1]
    win = e_buf.shape[-1]
    seq = ak.shape[-1]


    def wq_stream(b):
        def copy(col, beat, queue):
            half = pl.ds(8 * (col & 1), 8)
            for r in _on_queue(queue, _ROWS[beat]):
                at = (16 * r + (col >> 1), half)
                pltpu.make_async_copy(
                    (awq, bwq)[b].at[at], wq_buf.at[(b, *at)], wq_sem.at[b]
                ).start(priority=queue)

        return copy, 4, 32

    def kv_stream(j):
        def copy(sweep, beat, queue):
            col = _div6(sweep)
            part = sweep - 6 * col
            first = 128 * (part >> 1) + 4 * (part & 1) + (col >> 1)
            half = pl.ds(pl.multiple_of(8 * (col & 1), 8), 8)
            for r in _on_queue(queue, range(4 * beat, 4 * beat + 4)):
                pltpu.make_async_copy(
                    (ak, bk, av, bv)[j].at[first + 8 * r, half, pl.ds(seq - win, win)],
                    kv_buf.at[j, first + 8 * r, half],
                    kv_sem.at[j],
                ).start(priority=queue)

        return copy, 4, 48

    def wo_piece(third, r, col, sem, queue):
        tiles = pl.ds(8 * col, 8)
        pltpu.make_async_copy(
            (awo, bwo)[third // 3].at[third % 3, r, tiles], wo_buf.at[third, r, tiles], sem
        ).start(priority=queue)

    def wo_stream(b, late):
        rows, first, cols = (_LATE_ROWS, 22, 10) if late else (_ROWS, 0, 22)

        def copy(col, beat, queue):
            for r in _on_queue(queue, rows[beat]):
                wo_piece(3 * b + r // 5, r % 5, first + col, wo_sem.at[2 * b + late], queue)

        return copy, len(rows), cols

    def last_four(col, _, queue):
        for third in _on_queue(queue, range(4)):
            wo_piece(third, 4, 22 + col, end_sem.at[0], queue)

    def last_two(i, _, queue):
        for p in _on_queue(queue, range(4 * i, 4 * i + 4)):
            wo_piece(4 + p // 10, 4, 22 + p % 10, end_sem.at[1 + p // 5], queue)

    feed = _Feed([
        wq_stream(0), wq_stream(1),
        kv_stream(0), kv_stream(1), kv_stream(2), kv_stream(3),
        wo_stream(0, 0), wo_stream(0, 1), wo_stream(1, 0), wo_stream(1, 1),
        (last_four, 1, 10), (last_two, 1, 5),
    ])


    row = lax.broadcasted_iota(jnp.int32, (8, 128), 0)
    lane = lax.broadcasted_iota(jnp.int32, (8, 128), 1)

    def keep_own(t, x):
        d = lane + 128 * t - _HEAD_DIM * row
        return jnp.where(jnp.logical_and(d >= 0, d < _HEAD_DIM), x, 0.0)

    def queries(b, i, carry, step):
        x = jnp.broadcast_to(x_buf[b], (8, d_model))
        q = jnp.zeros((8, 3 * 128), _F32)
        for u in range(5):
            wt = _side_by_side(wq_buf[b, 48 * u:48 * (u + 1), i], 3)
            q = q + jnp.dot(x[:, 128 * u:128 * (u + 1)], wt, preferred_element_type=_F32)
            if u < 4:
                step()
        for j in range(3):
            t = 16 * j + i
            q_buf[b, t] = keep_own(t - 12 * _div6(t >> 1), q[:, 128 * j:128 * (j + 1)])
        return carry

    def scores(b, i, s, step):
        for u in range(2):
            t = 2 * i + u
            q = q_buf[b, t].astype(dtype)
            parts = []
            for lo in (0, win // 2):
                step()
                kt = kv_buf[b, pl.ds(8 * t, 8), :, lo:lo + win // 2].reshape(128, win // 2)
                parts.append(jnp.dot(q, kt, preferred_element_type=_F32))
            s = s + jnp.concatenate(parts, axis=1)
        return s

    def softmax(b, trip, g, carry):
        s = lax.fori_loop(0, 6, lambda i, s: trip(6 * g + i, s), jnp.zeros((8, win), _F32))
        s = s * _HEAD_DIM**-0.5
        e = jnp.exp(s - jnp.max(s, axis=-1, keepdims=True))
        e_buf[b, g] = e
        inv_buf[b, g] = jnp.broadcast_to(1.0 / jnp.sum(e, axis=-1, keepdims=True), (8, 128))
        return carry

    def values(b, n, i, carry, step):
        g = _div6((n * i) >> 1)
        e = e_buf[b, g].astype(dtype)
        for u in range(n):
            t = n * i + u
            step()
            vt = kv_buf[2 + b, pl.ds(8 * t, 8)].reshape(128, win)
            o = lax.dot_general(e, vt, (((1,), (1,)), ((), ())), preferred_element_type=_F32)
            o = keep_own(t - 12 * g, o * inv_buf[b, g])
            o_buf[48 * b + t] = jnp.broadcast_to(jnp.sum(o, axis=0, keepdims=True), (8, 128))
        return carry

    def project(third, j, acc):
        r, lo = divmod(80 * j, 256)
        tiles = wo_buf[third, r, lo:min(lo + 80, 256)]
        if lo + 80 > 256:
            tiles = jnp.concatenate([tiles, wo_buf[third, r + 1, 0:lo + 80 - 256]], axis=0)
        o = o_buf[16 * third + j].astype(dtype)
        return acc + jnp.dot(o, _side_by_side(tiles, 5), preferred_element_type=_F32)

    def outputs(b, blocks, per_trip, i, acc, step):
        n = len(blocks)
        for u, j in enumerate(blocks):
            for _ in range((u + 1) * per_trip // n - u * per_trip // n):
                step()
            acc = project(3 * b + i, j, acc)
        return acc


    feed.prime()
    pltpu.make_async_copy(ax, x_buf.at[0], x_sem).start()
    pltpu.make_async_copy(bx, x_buf.at[1], x_sem).start()
    feed.loop(30, 4)
    feed.loop(2, 4)
    _wait(x_buf, x_sem)
    for b in range(2):
        feed.loop(14 + 16 * b, 4)
        _wait(wq_buf.at[b], wq_sem.at[b])
        feed.loop(16, 4, functools.partial(queries, b))
        feed.loop(2, 4)
    for b in range(2):
        feed.loop(22, 4)
        _wait(kv_buf.at[b], kv_sem.at[b])
        trip = feed.trip(24, 4, functools.partial(scores, b))
        lax.fori_loop(0, 4, functools.partial(softmax, b, trip), None)
        feed.loop(2, 4)
    feed.loop(22, 4)
    _wait(kv_buf.at[2], kv_sem.at[2])
    feed.loop(24, 4, functools.partial(values, 0, 2))
    feed.loop(2, 4)
    feed.loop(4, 4)
    _wait(kv_buf.at[3], kv_sem.at[3])
    feed.loop(16, 4, functools.partial(values, 1, 3))
    feed.step(8)
    feed.loop(7, 3)
    feed.step(9)
    feed.loop(5, 4)
    early, late = pl.ds(0, 176), pl.ds(176, 80)
    _wait(wo_buf.at[0:3, :, early], wo_sem.at[0])
    _wait(wo_buf.at[0:3, 0:4, late], wo_sem.at[1])
    zero = jnp.zeros((8, d_model), _F32)
    acc_a = feed.loop(3, 20, functools.partial(outputs, 0, range(15), 20), zero)
    feed.step(8)
    feed.loop(4, 3)
    ready = [j for j in range(15) if 80 * j % 256 + 80 <= 176]
    _wait(wo_buf.at[3:6, :, early], wo_sem.at[2])
    acc_b = feed.loop(3, 3, functools.partial(outputs, 1, ready, 3), zero)
    feed.step(15)
    _wait(wo_buf.at[3:6, 0:4, late], wo_sem.at[3])
    rest = [(third, j) for third in range(3, 6) for j in range(15) if j not in ready]
    for u, (third, j) in enumerate(rest):
        if u % 2 == 0:
            feed.step()
        acc_b = project(third, j, acc_b)
    assert feed.done()

    o_cols = [
        jnp.broadcast_to(o_buf[16 * third + 15, 0:1].astype(dtype).astype(_F32), (128, 128)).T
        for third in (4, 5)
    ]
    _wait(wo_buf.at[0:4, 4, late], end_sem.at[0])
    for third in range(3):
        acc_a = project(third, 15, acc_a)
    acc_b = project(3, 15, acc_b)
    out_ref[:, 0:d_model] = acc_a[0:1].astype(dtype)
    part = [jnp.where(row == 0, acc_b[:, 128 * n:128 * (n + 1)], 0.0) for n in range(5)]
    for stage in range(4):
        u, half = divmod(stage, 2)
        tiles = pl.ds(176 + 40 * half, 40)
        _wait(wo_buf.at[4 + u, 4, tiles], end_sem.at[1 + stage])
        wt = wo_buf[4 + u, 4, tiles].astype(_F32).reshape(8, 5, 8, 128)
        o = o_cols[u][64 * half:64 * (half + 1)].reshape(8, 8, 128)
        for n in range(5):
            part[n] = part[n] + jnp.sum(wt[:, n] * o, axis=0)
    out_b = jnp.sum(jnp.concatenate(part, axis=1), axis=0, keepdims=True)
    out_ref[:, d_model:] = out_b.astype(dtype)


def _kernel(*refs):
    dma = pltpu.SemaphoreType.DMA
    pl.run_scoped(
        functools.partial(_attend, *refs),
        dma(()), dma((2,)), dma((4,)), dma((4,)), dma((5,)),
    )


@jax.jit
def pallas_concat_heads__sliding_block_cached__sliding_block_cached__decode_kernel(
    A_x: jax.Array,
    A_k_cache: jax.Array,
    A_v_cache: jax.Array,
    A_wq: jax.Array,
    A_wo: jax.Array,
    B_x: jax.Array,
    B_k_cache: jax.Array,
    B_v_cache: jax.Array,
    B_wq: jax.Array,
    B_wo: jax.Array,
):
    d_model = A_x.shape[-1]
    seq = A_k_cache.shape[2]
    win = min(4096, max(256, seq // 4))
    dtype = A_x.dtype
    assert A_x.shape == B_x.shape == (1, 1, 640)
    assert A_k_cache.shape == B_k_cache.shape == (1, _HEADS, seq, _HEAD_DIM)

    def seq_minor(cache):
        return jnp.swapaxes(cache, 2, 3).reshape(384, 16, seq)

    def tiled(w, *shape):
        rows, cols = w.shape
        w = w.reshape(rows // 8, 8, cols // 128, 128).transpose(0, 2, 1, 3)
        return w.reshape(*shape, 8, 128)

    out = pl.pallas_call(
        _kernel,
        out_shape=jax.ShapeDtypeStruct((1, 2 * d_model), dtype),
        in_specs=[pl.BlockSpec(memory_space=pltpu.HBM)] * 10,
        out_specs=pl.BlockSpec(memory_space=pltpu.VMEM),
        scratch_shapes=[
            pltpu.VMEM((2, 1, d_model), dtype),
            pltpu.VMEM((2, 240, 16, 8, 128), dtype),
            pltpu.VMEM((4, 384, 16, win), dtype),
            pltpu.VMEM((6, 5, 256, 8, 128), dtype),
            pltpu.VMEM((2, 48, 8, 128), _F32),
            pltpu.VMEM((2, 4, 8, win), _F32),
            pltpu.VMEM((2, 4, 8, 128), _F32),
            pltpu.VMEM((96, 8, 128), _F32),
        ],
        compiler_params=pltpu.CompilerParams(
            vmem_limit_bytes=100 * 1024 * 1024, disable_bounds_checks=True
        ),
    )(
        A_x.reshape(1, d_model), seq_minor(A_k_cache), seq_minor(A_v_cache),
        tiled(A_wq, 240, 16), tiled(A_wo, 3, 5, 256),
        B_x.reshape(1, d_model), seq_minor(B_k_cache), seq_minor(B_v_cache),
        tiled(B_wq, 240, 16), tiled(B_wo, 3, 5, 256),
    )
    return out.reshape(1, 1, 2 * d_model)
```

```python
import functools

import jax
import jax.numpy as jnp
from jax import lax
import jax.experimental.pallas as pl
import jax.experimental.pallas.tpu as pltpu

_HEADS, _HEAD_DIM = 32, 192
_F32 = jnp.float32

_LEAD = 8

_ROWS = ((0, 2, 4, 6), (8, 10, 12, 14), (1, 3, 5, 7), (9, 11, 13))
_LATE_ROWS = ((0, 2, 6, 8), (10, 12, 1, 3), (5, 7, 11, 13))


def _div6(i):
    return (i * 43) >> 8


def _on_queue(queue, pieces):
    return pieces[1:] if queue else pieces[:1]


def _wait(view, sem):
    pltpu.make_async_copy(view, view, sem).wait()


def _side_by_side(tiles, n):
    tiles = tiles.reshape(16, n, 8, 128)
    return jnp.concatenate([tiles[:, j].reshape(128, 128) for j in range(n)], axis=1)


class _Feed:
    def __init__(self, streams):
        self.streams = streams
        self.pos = 0

    def _locate(self, pos):
        for copy, beats, sweeps in self.streams:
            if pos < beats * sweeps:
                return copy, beats, pos, beats * sweeps - pos
            pos -= beats * sweeps
        return None

    def _issue(self, pos, queue):
        place = self._locate(pos)
        if place is not None:
            copy, beats, p, _ = place
            copy(p // beats, p % beats, queue)

    def prime(self):
        for pos in range(_LEAD):
            self._issue(pos, 1)

    def step(self, n=1):
        for _ in range(n):
            self._issue(self.pos + _LEAD, 1)
            self._issue(self.pos, 0)
            self.pos += 1

    def trip(self, trips, per_trip, work=None):
        places = ((1, self._locate(self.pos + _LEAD)), (0, self._locate(self.pos)))
        for _, (_, beats, _, left) in places:
            assert per_trip % beats == 0 and left >= trips * per_trip
        self.pos += trips * per_trip

        def body(i, carry):
            issued = 0

            def step():
                nonlocal issued
                for queue, (copy, beats, p, _) in places:
                    p += issued
                    copy(p // beats + i * (per_trip // beats), p % beats, queue)
                issued += 1

            if work is not None:
                carry = work(i, carry, step)
            assert issued <= per_trip
            while issued < per_trip:
                step()
            return carry

        return body

    def loop(self, trips, per_trip, work=None, carry=None):
        return lax.fori_loop(0, trips, self.trip(trips, per_trip, work), carry)

    def done(self):
        return self._locate(self.pos) is None


def _attend(
    ax, ak, av, awq, awo, bx, bk, bv, bwq, bwo, out_ref,
    x_buf, wq_buf, kv_buf, wo_buf, q_buf, e_buf, inv_buf, o_buf,
    x_sem, wq_sem, kv_sem, wo_sem, end_sem,
):
    dtype = x_buf.dtype
    d_model = x_buf.shape[-1]
    win = e_buf.shape[-1]
    seq = ak.shape[-1]


    def wq_stream(b):
        def copy(col, beat, queue):
            half = pl.ds(8 * (col & 1), 8)
            for r in _on_queue(queue, _ROWS[beat]):
                at = (16 * r + (col >> 1), half)
                pltpu.make_async_copy(
                    (awq, bwq)[b].at[at], wq_buf.at[(b, *at)], wq_sem.at[b]
                ).start(priority=queue)

        return copy, 4, 32

    def kv_stream(j):
        def copy(sweep, beat, queue):
            col = _div6(sweep)
            part = sweep - 6 * col
            first = 128 * (part >> 1) + 4 * (part & 1) + (col >> 1)
            half = pl.ds(pl.multiple_of(8 * (col & 1), 8), 8)
            for r in _on_queue(queue, range(4 * beat, 4 * beat + 4)):
                pltpu.make_async_copy(
                    (ak, bk, av, bv)[j].at[first + 8 * r, half, pl.ds(seq - win, win)],
                    kv_buf.at[j, first + 8 * r, half],
                    kv_sem.at[j],
                ).start(priority=queue)

        return copy, 4, 48

    def wo_piece(third, r, col, sem, queue):
        tiles = pl.ds(8 * col, 8)
        pltpu.make_async_copy(
            (awo, bwo)[third // 3].at[third % 3, r, tiles], wo_buf.at[third, r, tiles], sem
        ).start(priority=queue)

    def wo_stream(b, late):
        rows, first, cols = (_LATE_ROWS, 22, 10) if late else (_ROWS, 0, 22)

        def copy(col, beat, queue):
            for r in _on_queue(queue, rows[beat]):
                wo_piece(3 * b + r // 5, r % 5, first + col, wo_sem.at[2 * b + late], queue)

        return copy, len(rows), cols

    def last_four(col, _, queue):
        for third in _on_queue(queue, range(4)):
            wo_piece(third, 4, 22 + col, end_sem.at[0], queue)

    def last_two(i, _, queue):
        for p in _on_queue(queue, range(4 * i, 4 * i + 4)):
            wo_piece(4 + p // 10, 4, 22 + p % 10, end_sem.at[1 + p // 5], queue)

    feed = _Feed([
        wq_stream(0), wq_stream(1),
        kv_stream(0), kv_stream(1), kv_stream(2), kv_stream(3),
        wo_stream(0, 0), wo_stream(0, 1), wo_stream(1, 0), wo_stream(1, 1),
        (last_four, 1, 10), (last_two, 1, 5),
    ])


    row = lax.broadcasted_iota(jnp.int32, (8, 128), 0)
    lane = lax.broadcasted_iota(jnp.int32, (8, 128), 1)

    def keep_own(t, x):
        d = lane + 128 * t - _HEAD_DIM * row
        return jnp.where(jnp.logical_and(d >= 0, d < _HEAD_DIM), x, 0.0)

    def queries(b, i, carry, step):
        x = jnp.broadcast_to(x_buf[b], (8, d_model))
        q = jnp.zeros((8, 3 * 128), _F32)
        for u in range(5):
            wt = _side_by_side(wq_buf[b, 48 * u:48 * (u + 1), i], 3)
            q = q + jnp.dot(x[:, 128 * u:128 * (u + 1)], wt, preferred_element_type=_F32)
            if u < 4:
                step()
        for j in range(3):
            t = 16 * j + i
            q_buf[b, t] = keep_own(t - 12 * _div6(t >> 1), q[:, 128 * j:128 * (j + 1)])
        return carry

    def scores(b, i, s, step):
        for u in range(2):
            t = 2 * i + u
            q = q_buf[b, t].astype(dtype)
            parts = []
            for lo in (0, win // 2):
                step()
                kt = kv_buf[b, pl.ds(8 * t, 8), :, lo:lo + win // 2].reshape(128, win // 2)
                parts.append(jnp.dot(q, kt, preferred_element_type=_F32))
            s = s + jnp.concatenate(parts, axis=1)
        return s

    def softmax(b, trip, g, carry):
        s = lax.fori_loop(0, 6, lambda i, s: trip(6 * g + i, s), jnp.zeros((8, win), _F32))
        s = s * _HEAD_DIM**-0.5
        e = jnp.exp(s - jnp.max(s, axis=-1, keepdims=True))
        e_buf[b, g] = e
        inv_buf[b, g] = jnp.broadcast_to(1.0 / jnp.sum(e, axis=-1, keepdims=True), (8, 128))
        return carry

    def values(b, n, i, carry, step):
        g = _div6((n * i) >> 1)
        e = e_buf[b, g].astype(dtype)
        for u in range(n):
            t = n * i + u
            step()
            vt = kv_buf[2 + b, pl.ds(8 * t, 8)].reshape(128, win)
            o = lax.dot_general(e, vt, (((1,), (1,)), ((), ())), preferred_element_type=_F32)
            o = keep_own(t - 12 * g, o * inv_buf[b, g])
            o_buf[48 * b + t] = jnp.broadcast_to(jnp.sum(o, axis=0, keepdims=True), (8, 128))
        return carry

    def project(third, j, acc):
        r, lo = divmod(80 * j, 256)
        tiles = wo_buf[third, r, lo:min(lo + 80, 256)]
        if lo + 80 > 256:
            tiles = jnp.concatenate([tiles, wo_buf[third, r + 1, 0:lo + 80 - 256]], axis=0)
        o = o_buf[16 * third + j].astype(dtype)
        return acc + jnp.dot(o, _side_by_side(tiles, 5), preferred_element_type=_F32)

    def outputs(b, blocks, per_trip, i, acc, step):
        n = len(blocks)
        for u, j in enumerate(blocks):
            for _ in range((u + 1) * per_trip // n - u * per_trip // n):
                step()
            acc = project(3 * b + i, j, acc)
        return acc


    feed.prime()
    pltpu.make_async_copy(ax, x_buf.at[0], x_sem).start()
    pltpu.make_async_copy(bx, x_buf.at[1], x_sem).start()
    feed.loop(30, 4)
    feed.loop(2, 4)
    _wait(x_buf, x_sem)
    for b in range(2):
        feed.loop(14 + 16 * b, 4)
        _wait(wq_buf.at[b], wq_sem.at[b])
        feed.loop(16, 4, functools.partial(queries, b))
        feed.loop(2, 4)
    for b in range(2):
        feed.loop(22, 4)
        _wait(kv_buf.at[b], kv_sem.at[b])
        trip = feed.trip(24, 4, functools.partial(scores, b))
        lax.fori_loop(0, 4, functools.partial(softmax, b, trip), None)
        feed.loop(2, 4)
    feed.loop(22, 4)
    _wait(kv_buf.at[2], kv_sem.at[2])
    feed.loop(24, 4, functools.partial(values, 0, 2))
    feed.loop(2, 4)
    feed.loop(4, 4)
    _wait(kv_buf.at[3], kv_sem.at[3])
    feed.loop(16, 4, functools.partial(values, 1, 3))
    feed.step(8)
    feed.loop(7, 3)
    feed.step(9)
    feed.loop(5, 4)
    early, late = pl.ds(0, 176), pl.ds(176, 80)
    _wait(wo_buf.at[0:3, :, early], wo_sem.at[0])
    _wait(wo_buf.at[0:3, 0:4, late], wo_sem.at[1])
    zero = jnp.zeros((8, d_model), _F32)
    acc_a = feed.loop(3, 20, functools.partial(outputs, 0, range(15), 20), zero)
    feed.step(8)
    feed.loop(4, 3)
    ready = [j for j in range(15) if 80 * j % 256 + 80 <= 176]
    _wait(wo_buf.at[3:6, :, early], wo_sem.at[2])
    acc_b = feed.loop(3, 3, functools.partial(outputs, 1, ready, 3), zero)
    feed.step(16)
    _wait(wo_buf.at[3:6, 0:4, late], wo_sem.at[3])
    rest = [(third, j) for third in range(3, 6) for j in range(15) if j not in ready]
    for u, (third, j) in enumerate(rest):
        if u % 3 == 1:
            feed.step()
        acc_b = project(third, j, acc_b)
    assert feed.done()

    o_cols = [
        jnp.broadcast_to(o_buf[16 * third + 15, 0:1].astype(dtype).astype(_F32), (128, 128)).T
        for third in (4, 5)
    ]
    _wait(wo_buf.at[0:4, 4, late], end_sem.at[0])
    for third in range(3):
        acc_a = project(third, 15, acc_a)
    acc_b = project(3, 15, acc_b)
    out_ref[:, 0:d_model] = acc_a[0:1].astype(dtype)
    part = [jnp.where(row == 0, acc_b[:, 128 * n:128 * (n + 1)], 0.0) for n in range(5)]
    for stage in range(4):
        u, half = divmod(stage, 2)
        tiles = pl.ds(176 + 40 * half, 40)
        _wait(wo_buf.at[4 + u, 4, tiles], end_sem.at[1 + stage])
        wt = wo_buf[4 + u, 4, tiles].astype(_F32).reshape(8, 5, 8, 128)
        o = o_cols[u][64 * half:64 * (half + 1)].reshape(8, 8, 128)
        for n in range(5):
            part[n] = part[n] + jnp.sum(wt[:, n] * o, axis=0)
    out_b = jnp.sum(jnp.concatenate(part, axis=1), axis=0, keepdims=True)
    out_ref[:, d_model:] = out_b.astype(dtype)


def _kernel(*refs):
    dma = pltpu.SemaphoreType.DMA
    pl.run_scoped(
        functools.partial(_attend, *refs),
        dma(()), dma((2,)), dma((4,)), dma((4,)), dma((5,)),
    )


@jax.jit
def pallas_concat_heads__sliding_block_cached__sliding_block_cached__decode_kernel(
    A_x: jax.Array,
    A_k_cache: jax.Array,
    A_v_cache: jax.Array,
    A_wq: jax.Array,
    A_wo: jax.Array,
    B_x: jax.Array,
    B_k_cache: jax.Array,
    B_v_cache: jax.Array,
    B_wq: jax.Array,
    B_wo: jax.Array,
):
    d_model = A_x.shape[-1]
    seq = A_k_cache.shape[2]
    win = min(4096, max(256, seq // 4))
    dtype = A_x.dtype
    assert A_x.shape == B_x.shape == (1, 1, 640)
    assert A_k_cache.shape == B_k_cache.shape == (1, _HEADS, seq, _HEAD_DIM)

    def seq_minor(cache):
        return jnp.swapaxes(cache, 2, 3).reshape(384, 16, seq)

    def tiled(w, *shape):
        rows, cols = w.shape
        w = w.reshape(rows // 8, 8, cols // 128, 128).transpose(0, 2, 1, 3)
        return w.reshape(*shape, 8, 128)

    out = pl.pallas_call(
        _kernel,
        out_shape=jax.ShapeDtypeStruct((1, 2 * d_model), dtype),
        in_specs=[pl.BlockSpec(memory_space=pltpu.HBM)] * 10,
        out_specs=pl.BlockSpec(memory_space=pltpu.VMEM),
        scratch_shapes=[
            pltpu.VMEM((2, 1, d_model), dtype),
            pltpu.VMEM((2, 240, 16, 8, 128), dtype),
            pltpu.VMEM((4, 384, 16, win), dtype),
            pltpu.VMEM((6, 5, 256, 8, 128), dtype),
            pltpu.VMEM((2, 48, 8, 128), _F32),
            pltpu.VMEM((2, 4, 8, win), _F32),
            pltpu.VMEM((2, 4, 8, 128), _F32),
            pltpu.VMEM((96, 8, 128), _F32),
        ],
        compiler_params=pltpu.CompilerParams(vmem_limit_bytes=100 * 1024 * 1024),
    )(
        A_x.reshape(1, d_model), seq_minor(A_k_cache), seq_minor(A_v_cache),
        tiled(A_wq, 240, 16), tiled(A_wo, 3, 5, 256),
        B_x.reshape(1, d_model), seq_minor(B_k_cache), seq_minor(B_v_cache),
        tiled(B_wq, 240, 16), tiled(B_wo, 3, 5, 256),
    )
    return out.reshape(1, 1, 2 * d_model)
```
